```python
import os as _os
_os.environ.setdefault("JAX_PLATFORMS", "cpu")
import jax
import jax.numpy as jnp

def _softmax(x, axis=-1):
    return jax.nn.softmax(x, axis=axis)
def _gelu(x):
    return jax.nn.gelu(x, approximate=True)
def _silu(x):
    return jax.nn.silu(x)
def _sigmoid(x):
    return jax.nn.sigmoid(x)
def _layernorm(x, axis=-1, eps=1e-5):
    m = jnp.mean(x, axis=axis, keepdims=True)
    v = jnp.var(x, axis=axis, keepdims=True)
    return (x - m) / jnp.sqrt(v + eps)
def _scatter_add(tgt, idx, src, axis=0):
    return tgt.at[idx].add(src)
def _segment_sum(src, seg, n):
    return jax.ops.segment_sum(src, seg, n)
class _Rng:
    def __init__(self, key):
        self._k = key
    def _next(self):
        self._k, sub = jax.random.split(self._k)
        return sub
    def normal(self, shape):
        return jax.random.normal(self._next(), shape, dtype=jnp.bfloat16)
    def randint(self, lo, hi, shape):
        return jax.random.randint(self._next(), shape, lo, hi, dtype=jnp.int32)
    def uniform(self, shape, lo=0.0, hi=1.0):
        return jax.random.uniform(self._next(), shape, jnp.bfloat16, lo, hi)
    def permutation(self, n):
        return jax.random.permutation(self._next(), n)


kernel_name = 'sequential_preLN__mha_block__swiglu_ffn__prompt'

def setup_inputs():
    _rng = _Rng(jax.random.key(int.from_bytes(__import__("os").urandom(4), "little")))
    _w = (lambda a: (lambda t: t.astype(jnp.bfloat16) if jnp.issubdtype(t.dtype, jnp.floating) else t)(jnp.asarray(a)))
    def _A_setup():
        B, S, D, H = 1, 2048, 640, 32
        return {
            "x": _w((lambda *s: _rng.normal(s) * 0.05)(B, S, D)),
            "wqkv": _w((lambda *s: _rng.normal(s) * 0.05)(D, 3 * D)),
            "wo": _w((lambda *s: _rng.normal(s) * 0.05)(D, D)),
        }
    _A_in = _A_setup()

    def _B_setup():
        B, S, D, F = 1, 2048, 640, 1728
        return {
            "x": _w((lambda *s: _rng.normal(s) * 0.05)(B, S, D)),
            "w_gate": _w((lambda *s: _rng.normal(s) * 0.05)(D, F)),
            "w_up": _w((lambda *s: _rng.normal(s) * 0.05)(D, F)),
            "w_down": _w((lambda *s: _rng.normal(s) * 0.05)(F, D)),
        }
    _B_in = _B_setup()

    return {
        "A_x": _A_in["x"],
        "A_wqkv": _A_in["wqkv"],
        "A_wo": _A_in["wo"],
        "B_x": _B_in["x"],
        "B_w_gate": _B_in["w_gate"],
        "B_w_up": _B_in["w_up"],
        "B_w_down": _B_in["w_down"],
    }

def reference(A_x, A_wqkv, A_wo, B_x, B_w_gate, B_w_up, B_w_down):
    def _A_ref(x, wqkv, wo):
        B, S, D = x.shape
        H = 32
        Dh = D // H
        qkv = (lambda x, *d: x.transpose(*d))((x @ wqkv).reshape(B, S, 3, H, Dh), 2, 0, 3, 1, 4)
        q, k, v = qkv[0], qkv[1], qkv[2]
        scores = jnp.einsum("bhqd,bhkd->bhqk", q, k) * (Dh ** -0.5)
        p = _softmax(scores, axis=-1)
        o = jnp.einsum("bhqk,bhkd->bhqd", p, v)
        return (lambda x, *d: x.transpose(*d))(o, 0, 2, 1, 3).reshape(B, S, D) @ wo

    def _B_ref(x, w_gate, w_up, w_down):
        g = _silu(x @ w_gate)
        u = x @ w_up
        return (g * u) @ w_down

    x = A_x
    h = x + _A_ref(_layernorm(x, axis=-1), A_wqkv, A_wo)
    h2 = h + _B_ref(_layernorm(h, axis=-1), B_w_gate, B_w_up, B_w_down)
    return h2
```

```python
import functools
import math

import jax
import jax.numpy as jnp
from jax import lax
import jax.experimental.pallas as pl
import jax.experimental.pallas.tpu as pltpu

_H = 32
_EPS = 1e-5
_HPW = 6
_NW = 6

_BF16 = jnp.bfloat16
_F32 = jnp.float32


def _win_start_static(w, D, Dh):
    return min(((_HPW * Dh * w) // 16) * 16, D - 128)


def _layernorm_f32(x):
    m = jnp.mean(x, axis=-1, keepdims=True)
    xc = x - m
    v = jnp.mean(xc * xc, axis=-1, keepdims=True)
    return xc * lax.rsqrt(v + _EPS)


def _kernel(x_ref, wqkv_ref, wo_hbm, wg_hbm, wu_hbm, wd_hbm,
            o_ref,
            wo_ref, wg_ref, wu_ref, wd_ref, sems,
            k_scr, qT_scr, vT_scr, s0, s1, m0, m1, oT_scr,
            *, S, D, F, tq, ck, unroll, tp, fc):
    Dh = D // _H
    n_qt = S // tq
    nck = S // ck
    t = pl.program_id(0)
    sb = (s0, s1)
    mb = (m0, m1)

    def weight_copies():
        return [
            pltpu.make_async_copy(wo_hbm, wo_ref, sems.at[0]),
            pltpu.make_async_copy(wg_hbm, wg_ref, sems.at[1]),
            pltpu.make_async_copy(wu_hbm, wu_ref, sems.at[2]),
            pltpu.make_async_copy(wd_hbm, wd_ref, sems.at[3]),
        ]

    def q_rhs(tt, h):
        w = jnp.minimum(h // _HPW, _NW - 1)
        w0 = jnp.minimum(((_HPW * Dh * w) // 16) * 16, D - 128)
        w0 = pl.multiple_of(w0, 16)
        qt = qT_scr[tt, pl.ds(w0, 128), :]
        lo = Dh * h - w0
        r = lax.broadcasted_iota(jnp.int32, (128, tq), 0)
        mask = jnp.logical_and(r >= lo, r < lo + Dh)
        return w, jnp.where(mask, qt, jnp.zeros_like(qt))

    def v_lhs(h):
        blk = pl.multiple_of(((Dh * h) // 16) * 16, 16)
        off = Dh * h - blk
        vt = vT_scr[pl.ds(blk, 32), :]
        r = lax.broadcasted_iota(jnp.int32, (32, S), 0)
        mask = jnp.logical_and(r >= off, r < off + Dh)
        return blk, off, jnp.where(mask, vt, jnp.ones_like(vt))

    def a_chunk(w, rhs, c, buf, mrun):
        s = jnp.dot(k_scr[w, c * ck:(c + 1) * ck, :], rhs,
                    preferred_element_type=_F32)
        sb[buf][c * ck:(c + 1) * ck, :] = s
        mm = jnp.max(s.reshape(ck // 8, 8, tq), axis=0)
        return mm if mrun is None else jnp.maximum(mrun, mm)

    def b_chunk(vl, c, buf, m, acc):
        p = jnp.exp2(sb[buf][c * ck:(c + 1) * ck, :] - m).astype(_BF16)
        o = jnp.dot(vl[:, c * ck:(c + 1) * ck], p, preferred_element_type=_F32)
        return o if acc is None else acc + o

    def b_finish(blk, off, acc):
        l = jnp.where(off == 12, acc[0:1, :], acc[31:32, :])
        on = acc * (1.0 / l)
        r = lax.broadcasted_iota(jnp.int32, (32, tq), 0)
        mask = jnp.logical_and(r >= off, r < off + Dh)
        old = oT_scr[pl.ds(blk, 32), :]
        oT_scr[pl.ds(blk, 32), :] = jnp.where(mask, on, old)

    @pl.when(t == 0)
    def _phase0():
        for cp in weight_copies():
            cp.start()
        oT_scr[...] = jnp.zeros_like(oT_scr)
        wk_win = jnp.concatenate(
            [wqkv_ref[:, D + _win_start_static(w, D, Dh): D + _win_start_static(w, D, Dh) + 128]
             for w in range(_NW)], axis=1)
        wqT = wqkv_ref[:, 0:D].astype(_F32).T.astype(_BF16)
        wvT = wqkv_ref[:, 2 * D:3 * D].astype(_F32).T.astype(_BF16)
        qscale = (Dh ** -0.5) * math.log2(math.e)
        for i in range(S // tp):
            rows = slice(i * tp, (i + 1) * tp)
            xn = _layernorm_f32(x_ref[rows, :].astype(_F32))
            xnb = xn.astype(_BF16)
            xnT = xn.T.astype(_BF16)
            kk = jnp.dot(xnb, wk_win, preferred_element_type=_F32)
            for w in range(_NW):
                k_scr[w, rows, :] = kk[:, w * 128:(w + 1) * 128].astype(_BF16)
            qT = jnp.dot(wqT, xnT, preferred_element_type=_F32) * qscale
            for j in range(tp // tq if tp >= tq else 1):
                if tp >= tq:
                    qT_scr[i * (tp // tq) + j] = qT[:, j * tq:(j + 1) * tq].astype(_BF16)
                else:
                    c0 = (i * tp) % tq
                    qT_scr[(i * tp) // tq, :, c0:c0 + tp] = qT.astype(_BF16)
            vT = jnp.dot(wvT, xnT, preferred_element_type=_F32)
            vT_scr[:, rows] = vT.astype(_BF16)
        w, rhs = q_rhs(0, 0)
        mrun = None
        for c in range(nck):
            mrun = a_chunk(w, rhs, c, 0, mrun)
        m0[...] = jnp.max(mrun, axis=0, keepdims=True)

    def body(g, carry):
        for j in range(unroll):
            h = g * unroll + j
            un = t * _H + h + 1
            un = jnp.minimum(un, n_qt * _H - 1)
            tn = un // _H
            hn = un % _H
            cur = j % 2
            nxt = 1 - cur
            w, rhs = q_rhs(tn, hn)
            blk, off, vl = v_lhs(h)
            m = mb[cur][...]
            mrun = None
            acc = None
            for c in range(nck):
                mrun = a_chunk(w, rhs, c, nxt, mrun)
                acc = b_chunk(vl, c, cur, m, acc)
            mb[nxt][...] = jnp.max(mrun, axis=0, keepdims=True)
            b_finish(blk, off, acc)
        return carry

    lax.fori_loop(0, _H // unroll, body, 0)

    @pl.when(t == 0)
    def _wait_weights():
        for cp in weight_copies():
            cp.wait()

    o = oT_scr[...].T.astype(_BF16)
    row0 = pl.multiple_of(t * tq, tq)
    xt = x_ref[pl.ds(row0, tq), :].astype(_F32)
    h1 = xt + jnp.dot(o, wo_ref[...], preferred_element_type=_F32)
    hn = _layernorm_f32(h1).astype(_BF16)
    y = h1
    f0 = 0
    while f0 < F:
        f1 = min(f0 + fc, F)
        g = jnp.dot(hn, wg_ref[:, f0:f1], preferred_element_type=_F32)
        u = jnp.dot(hn, wu_ref[:, f0:f1], preferred_element_type=_F32)
        a = (g * jax.nn.sigmoid(g) * u).astype(_BF16)
        y = y + jnp.dot(a, wd_ref[f0:f1, :], preferred_element_type=_F32)
        f0 = f1
    o_ref[...] = y.astype(o_ref.dtype)


def _build(S, D, F, dtype, tq=512, ck=128, unroll=2, tp=512, fc=256):
    n_qt = S // tq
    kern = functools.partial(_kernel, S=S, D=D, F=F, tq=tq, ck=ck, unroll=unroll, tp=tp, fc=fc)
    return pl.pallas_call(
        kern,
        grid=(n_qt,),
        in_specs=[
            pl.BlockSpec((S, D), lambda t: (0, 0)),
            pl.BlockSpec((D, 3 * D), lambda t: (0, 0)),
            pl.BlockSpec(memory_space=pl.ANY),
            pl.BlockSpec(memory_space=pl.ANY),
            pl.BlockSpec(memory_space=pl.ANY),
            pl.BlockSpec(memory_space=pl.ANY),
        ],
        out_specs=pl.BlockSpec((tq, D), lambda t: (t, 0)),
        out_shape=jax.ShapeDtypeStruct((S, D), dtype),
        scratch_shapes=[
            pltpu.VMEM((D, D), _BF16),
            pltpu.VMEM((D, F), _BF16),
            pltpu.VMEM((D, F), _BF16),
            pltpu.VMEM((F, D), _BF16),
            pltpu.SemaphoreType.DMA((4,)),
            pltpu.VMEM((_NW, S, 128), _BF16),
            pltpu.VMEM((n_qt, D, tq), _BF16),
            pltpu.VMEM((D, S), _BF16),
            pltpu.VMEM((S, tq), _F32),
            pltpu.VMEM((S, tq), _F32),
            pltpu.VMEM((1, tq), _F32),
            pltpu.VMEM((1, tq), _F32),
            pltpu.VMEM((D, tq), _F32),
        ],
        compiler_params=pltpu.CompilerParams(
            dimension_semantics=("arbitrary",),
            vmem_limit_bytes=100 * 1024 * 1024,
        ),
        name="preln_mha_swiglu",
    )


@jax.jit
def pallas_sequential_preLN__mha_block__swiglu_ffn__prompt_kernel(
    A_x: jax.Array,
    A_wqkv: jax.Array,
    A_wo: jax.Array,
    B_x: jax.Array,
    B_w_gate: jax.Array,
    B_w_up: jax.Array,
    B_w_down: jax.Array,
):
    B, S, D = A_x.shape
    F = B_w_gate.shape[1]
    assert B == 1 and D == 640 and S % 512 == 0
    x = A_x.reshape(S, D)
    out = _build(S, D, F, A_x.dtype)(x, A_wqkv, A_wo, B_w_gate, B_w_up, B_w_down)
    return out.reshape(B, S, D)
```

```python
import functools
import math

import jax
import jax.numpy as jnp
from jax import lax
import jax.experimental.pallas as pl
import jax.experimental.pallas.tpu as pltpu

_H = 32
_EPS = 1e-5
_G = 4
_NG = _H // _G

_BF16 = jnp.bfloat16
_F32 = jnp.float32
_NT = (((1,), (1,)), ((), ()))
_NN = (((1,), (0,)), ((), ()))


def _layernorm_f32(x):
    m = jnp.mean(x, axis=-1, keepdims=True)
    xc = x - m
    v = jnp.mean(xc * xc, axis=-1, keepdims=True)
    return xc * lax.rsqrt(v + _EPS)


def _kernel(x_hbm, wqkv_hbm, wo_hbm, wgT_hbm, wuT_hbm, wd_hbm,
            out_hbm,
            x_ref, wqkv_ref, wo_ref, wgT_ref, wuT_ref, wd_ref,
            x_sems, w_sems, o_sems, zero_smem,
            xn_scr, k_scr, qT_scr, vT_scr, s0, s1, m0, m1, oT_scr,
            hn_scr, h1_scr, out_scr,
            *, S, D, F, tq, ck, unroll, tp, rs, fc, mid, skew):
    Dh = D // _H
    n_qt = S // tq
    n_tp = S // tp
    n_rs = S // rs
    nck = S // ck
    GW = _G * Dh
    sb = (s0, s1)
    mb = (m0, m1)

    def x_copy(i):
        rows = pl.ds(pl.multiple_of(i * tp, tp), tp)
        return pltpu.make_async_copy(x_hbm.at[rows, :], x_ref.at[rows, :], x_sems.at[i])

    def w_copy(i):
        cols = pl.ds(i * D, D)
        return pltpu.make_async_copy(wqkv_hbm.at[:, cols], wqkv_ref.at[:, cols], w_sems.at[5 + i])

    late_copies = [
        pltpu.make_async_copy(wo_hbm, wo_ref, w_sems.at[1]),
        pltpu.make_async_copy(wgT_hbm, wgT_ref, w_sems.at[2]),
        pltpu.make_async_copy(wuT_hbm, wuT_ref, w_sems.at[3]),
        pltpu.make_async_copy(wd_hbm, wd_ref, w_sems.at[4]),
    ]

    def out_copy(r):
        rows = pl.ds(pl.multiple_of(r * rs, rs), rs)
        return pltpu.make_async_copy(out_scr.at[rows, :], out_hbm.at[rows, :], o_sems.at[r])

    x_copy(0).start()
    w_copy(0).start()
    zero_smem[0] = 0
    s1[...] = jnp.zeros_like(s1)
    m1[...] = jnp.zeros_like(m1)
    oT_scr[0:tq // rs, 0:GW, :] = jnp.zeros((tq // rs, GW, rs), _F32)

    def ln1(i):
        rows = pl.ds(pl.multiple_of(i * tp, tp), tp)
        xn_scr[rows, :] = _layernorm_f32(x_ref[rows, :].astype(_F32)).astype(_BF16)

    qscale = (Dh ** -0.5) * math.log2(math.e)

    def proj_q(i, xnb):
        q = jnp.dot(xnb, wqkv_ref[:, 0:D], preferred_element_type=_F32) * qscale
        qT_scr[i] = q.astype(_BF16).T

    def proj_v(i, xnb):
        v = jnp.dot(xnb, wqkv_ref[:, 2 * D:3 * D], preferred_element_type=_F32)
        vT_scr[i] = v.astype(_BF16).T.astype(_F32)

    def proj_k(i, xnb):
        rows = pl.ds(pl.multiple_of(i * tp, tp), tp)
        kk = jnp.dot(xnb, wqkv_ref[:, D:2 * D], preferred_element_type=_F32).astype(_BF16)
        kk = jnp.concatenate([kk, jnp.zeros((tp, 128), _BF16)], axis=1)
        for w in range(_NG):
            k_scr[w, rows, :] = kk[:, w * GW:w * GW + 128]

    x_copy(0).wait()
    ln1(0)
    w_copy(0).wait()
    w_copy(2).start()
    proj_q(0, xn_scr[0:tp, :])
    w_copy(2).wait()
    w_copy(1).start()
    x_copy(1).start()
    proj_v(0, xn_scr[0:tp, :])
    w_copy(1).wait()
    x_copy(1).wait()
    for i in range(2, n_tp):
        x_copy(i).start()
    proj_k(0, xn_scr[0:tp, :])
    ln1(1)

    def proj(i, carry):
        @pl.when(i + 1 < n_tp)
        def _():
            x_copy(i + 1).wait()

        xnb = xn_scr[pl.ds(pl.multiple_of(i * tp, tp), tp), :]
        proj_q(i, xnb)
        proj_v(i, xnb)
        proj_k(i, xnb)
        ln1(jnp.minimum(i + 1, n_tp - 1))
        return carry

    lax.fori_loop(1, n_tp, proj, 0)
    for cp in late_copies:
        cp.start()

    def head_mask(j, width):
        off = Dh * j - 16 * j
        r = lax.broadcasted_iota(jnp.int32, (32, width), 0)
        return jnp.logical_and(r >= off, r < off + Dh)

    def q_rhs(tt, g, j):
        r0 = pl.multiple_of(g * GW + 16 * j, 16)
        npc = tq // tp
        qt = [qT_scr[tt * npc + i, pl.ds(r0, 32), :] for i in range(npc)]
        qt = qt[0] if npc == 1 else jnp.concatenate(qt, axis=1)
        qt = jnp.where(head_mask(j, tq), qt, jnp.zeros_like(qt))
        parts = []
        if j > 0:
            parts.append(jnp.zeros((16 * j, tq), _BF16))
        parts.append(qt)
        parts.append(jnp.zeros((128 - 32 - 16 * j, tq), _BF16))
        return jnp.concatenate(parts, axis=0)

    def a_chunk(g, rhs, c, buf, mrun):
        s = jnp.dot(k_scr[g, c * ck:(c + 1) * ck, :], rhs,
                    preferred_element_type=_F32)
        sb[buf][0, c * ck:(c + 1) * ck, :] = s
        mm = jnp.max(s.reshape(ck // 8, 8, tq), axis=0)
        return mm if mrun is None else jnp.maximum(mrun, mm)

    def v_block(j):
        b0 = ((Dh * j) // 8) * 8
        return b0, Dh * j - b0

    def b_chunk(g, j, c, buf, z, m, acc):
        p = jnp.exp2(sb[buf][z, c * ck:(c + 1) * ck, :] - m).astype(_BF16)
        b0, off = v_block(j)
        r0 = pl.multiple_of(g * GW + b0, 8)
        c0 = (c * ck) % tp
        vt = vT_scr[(c * ck) // tp, pl.ds(r0, 24), c0:c0 + ck]
        r = lax.broadcasted_iota(jnp.int32, (24, ck), 0)
        vl = jnp.where(jnp.logical_and(r >= off, r < off + Dh), vt, 1.0)
        o = lax.dot_general(vl, p, _NN, preferred_element_type=_F32)
        return o if acc is None else acc + o

    def b_finish(t, g, j, acc):
        b0, off = v_block(j)
        l = acc[0:1, :] if off > 0 else acc[23:24, :]
        on = acc * (1.0 / l)
        r0 = pl.multiple_of(g * GW + b0, 8)
        npr = tq // rs
        for i in range(npr):
            lo = on[0:8, i * rs:(i + 1) * rs]
            if off > 0:
                r = lax.broadcasted_iota(jnp.int32, (8, rs), 0)
                lo = jnp.where(r >= off, lo, oT_scr[t * npr + i, pl.ds(r0, 8), :])
            oT_scr[t * npr + i, pl.ds(r0, 8), :] = lo
            oT_scr[t * npr + i, pl.ds(r0 + 8, 16), :] = on[8:24, i * rs:(i + 1) * rs]

    z = zero_smem[0]
    gpi = unroll // _G
    n_units = n_qt * _NG

    def step(a_unit, b_unit, par):
        if a_unit is not None:
            rhs = q_rhs(*a_unit)
        m = mb[1 - par][...]
        mrun = None
        acc = None
        for c in range(nck + skew):
            if c < nck and a_unit is not None:
                mrun = a_chunk(a_unit[1], rhs, c, par, mrun)
            if c >= skew:
                acc = b_chunk(b_unit[1], b_unit[2], c - skew, 1 - par, z, m, acc)
        if a_unit is not None:
            mb[par][...] = jnp.max(mrun, axis=0, keepdims=True)
        b_finish(*b_unit, acc)

    def attn_body(it, carry):
        for gg in range(gpi):
            u = it * gpi + gg
            t = u // _NG
            g = u % _NG
            for j in range(_G):
                if j > 0:
                    b_unit = (t, g, j - 1)
                else:
                    up = jnp.maximum(u - 1, 0)
                    b_unit = (up // _NG, up % _NG, _G - 1)
                step((t, g, j), b_unit, j % 2)
        return carry

    lax.fori_loop(0, n_units // gpi, attn_body, 0)

    for cp in late_copies:
        cp.wait()

    def out_proj(r):
        rows = pl.ds(pl.multiple_of(r * rs, rs), rs)
        o = oT_scr[r].astype(_BF16).T
        h1 = x_ref[rows, :].astype(_F32) + jnp.dot(o, wo_ref[...], preferred_element_type=_F32)
        hn_scr[rows, :] = _layernorm_f32(h1).astype(_BF16)
        h1_scr[rows, :] = h1

    def ffn(r, mid_work):
        rows = pl.ds(pl.multiple_of(r * rs, rs), rs)
        hn = hn_scr[rows, :]
        y = h1_scr[rows, :]
        f0 = 0
        while f0 < F:
            if f0 == mid * fc:
                mid_work()
            f1 = min(f0 + fc, F)
            g = lax.dot_general(hn, wgT_ref[f0:f1, :], _NT, preferred_element_type=_F32)
            u = lax.dot_general(hn, wuT_ref[f0:f1, :], _NT, preferred_element_type=_F32)
            a = (g * jax.nn.sigmoid(g) * u).astype(_BF16)
            y = y + jnp.dot(a, wd_ref[f0:f1, :], preferred_element_type=_F32)
            f0 = f1
        out_scr[rows, :] = y.astype(out_scr.dtype)

    out_proj(0)
    step(None, (n_qt - 1, _NG - 1, _G - 1), 0)

    def ffn_body(r, carry):
        ffn(r, lambda: out_proj(jnp.minimum(r + 1, n_rs - 1)))
        out_copy(r).start()
        return carry

    lax.fori_loop(0, n_rs, ffn_body, 0)
    for r in range(n_rs):
        out_copy(r).wait()


def _build(S, D, F, dtype, tq=512, ck=128, unroll=8, tp=512, rs=256, fc=256, mid=4, skew=1):
    assert tq % tp == 0 and tp % ck == 0 and tq % rs == 0
    kern = functools.partial(_kernel, S=S, D=D, F=F, tq=tq, ck=ck, unroll=unroll, tp=tp,
                             rs=rs, fc=fc, mid=mid, skew=skew)
    return pl.pallas_call(
        kern,
        in_specs=[pl.BlockSpec(memory_space=pl.ANY)] * 6,
        out_specs=pl.BlockSpec(memory_space=pl.ANY),
        out_shape=jax.ShapeDtypeStruct((S, D), dtype),
        scratch_shapes=[
            pltpu.VMEM((S, D), _BF16),
            pltpu.VMEM((D, 3 * D), _BF16),
            pltpu.VMEM((D, D), _BF16),
            pltpu.VMEM((F, D), _BF16),
            pltpu.VMEM((F, D), _BF16),
            pltpu.VMEM((F, D), _BF16),
            pltpu.SemaphoreType.DMA((S // tp,)),
            pltpu.SemaphoreType.DMA((8,)),
            pltpu.SemaphoreType.DMA((S // rs,)),
            pltpu.SMEM((1,), jnp.int32),
            pltpu.VMEM((S, D), _BF16),
            pltpu.VMEM((_NG, S, 128), _BF16),
            pltpu.VMEM((S // tp, D, tp), _BF16),
            pltpu.VMEM((S // tp, D, tp), _F32),
            pltpu.VMEM((1, S, tq), _F32),
            pltpu.VMEM((1, S, tq), _F32),
            pltpu.VMEM((1, tq), _F32),
            pltpu.VMEM((1, tq), _F32),
            pltpu.VMEM((S // rs, D, rs), _F32),
            pltpu.VMEM((S, D), _BF16),
            pltpu.VMEM((S, D), _F32),
            pltpu.VMEM((S, D), dtype),
        ],
        compiler_params=pltpu.CompilerParams(
            vmem_limit_bytes=100 * 1024 * 1024,
        ),
        name="preln_mha_swiglu",
    )


@jax.jit
def pallas_sequential_preLN__mha_block__swiglu_ffn__prompt_kernel(
    A_x: jax.Array,
    A_wqkv: jax.Array,
    A_wo: jax.Array,
    B_x: jax.Array,
    B_w_gate: jax.Array,
    B_w_up: jax.Array,
    B_w_down: jax.Array,
):
    B, S, D = A_x.shape
    F = B_w_gate.shape[1]
    assert B == 1 and D == 640 and S % 512 == 0
    x = A_x.reshape(S, D)
    out = _build(S, D, F, A_x.dtype)(x, A_wqkv, A_wo, B_w_gate.T, B_w_up.T, B_w_down)
    return out.reshape(B, S, D)
```

```python
import functools
import math

import jax
import jax.numpy as jnp
from jax import lax
import jax.experimental.pallas as pl
import jax.experimental.pallas.tpu as pltpu

_H = 32
_EPS = 1e-5
_G = 4
_NG = _H // _G

_BF16 = jnp.bfloat16
_F32 = jnp.float32
_NT = (((1,), (1,)), ((), ()))
_NN = (((1,), (0,)), ((), ()))


def _layernorm_f32(x):
    m = jnp.mean(x, axis=-1, keepdims=True)
    xc = x - m
    v = jnp.mean(xc * xc, axis=-1, keepdims=True)
    return xc * lax.rsqrt(v + _EPS)


def _kernel(x_hbm, wqkv_hbm, wo_hbm, wgT_hbm, wuT_hbm, wd_hbm,
            out_hbm,
            x_ref, wqkv_ref, wo_ref, wgT_ref, wuT_ref, wd_ref,
            x_sems, w_sems, o_sems, zero_smem,
            xn_scr, k_scr, qT_scr, vT_scr, s0, s1, m0, m1, oT_scr,
            hn_scr, h1_scr, out_scr,
            *, S, D, F, tq, ck, unroll, tp, tp0, rs, rt, fc, mid, skew):
    Dh = D // _H
    n_qt = S // tq
    n_tp = S // tp
    n_rs = S // rs
    nck = S // ck
    GW = _G * Dh
    sb = (s0, s1)
    mb = (m0, m1)

    def x_copy(i):
        rows = pl.ds(pl.multiple_of(i * tp, tp), tp)
        return pltpu.make_async_copy(x_hbm.at[rows, :], x_ref.at[rows, :], x_sems.at[i])

    def w_copy(i):
        cols = pl.ds(i * D, D)
        return pltpu.make_async_copy(wqkv_hbm.at[:, cols], wqkv_ref.at[:, cols], w_sems.at[i])

    late_copies = [
        pltpu.make_async_copy(wo_hbm, wo_ref, w_sems.at[3]),
        pltpu.make_async_copy(wgT_hbm, wgT_ref, w_sems.at[4]),
        pltpu.make_async_copy(wuT_hbm, wuT_ref, w_sems.at[5]),
        pltpu.make_async_copy(wd_hbm, wd_ref, w_sems.at[6]),
    ]

    def out_copy(row0, n, sem):
        rows = pl.ds(pl.multiple_of(row0, n), n)
        return pltpu.make_async_copy(out_scr.at[rows, :], out_hbm.at[rows, :], o_sems.at[sem])

    x_copy(0).start()
    w_copy(0).start()
    zero_smem[0] = 0

    def zero_fill(i, carry):
        s1[0, pl.ds(pl.multiple_of(i * ck, ck), ck), :] = jnp.zeros((ck, tq), _F32)
        return carry

    lax.fori_loop(0, nck, zero_fill, 0)
    m1[...] = jnp.zeros_like(m1)
    oT_scr[0:tq // rs, 0:GW, :] = jnp.zeros((tq // rs, GW, rs), _F32)

    def ln1(i):
        rows = pl.ds(pl.multiple_of(i * tp, tp), tp)
        xn_scr[rows, :] = _layernorm_f32(x_ref[rows, :].astype(_F32)).astype(_BF16)

    qscale = (Dh ** -0.5) * math.log2(math.e)

    def proj_q(i, xnb, c0=0):
        n = xnb.shape[0]
        q = jnp.dot(xnb, wqkv_ref[:, 0:D], preferred_element_type=_F32) * qscale
        qT_scr[i, :, c0:c0 + n] = q.astype(_BF16).T

    def proj_v(i, xnb, c0=0):
        n = xnb.shape[0]
        v = jnp.dot(xnb, wqkv_ref[:, 2 * D:3 * D], preferred_element_type=_F32)
        vT_scr[i, :, c0:c0 + n] = v.astype(_BF16).T.astype(_F32)

    def proj_k(i, xnb, c0=0):
        n = xnb.shape[0]
        rows = pl.ds(pl.multiple_of(i * tp + c0, 128), n)
        kk = jnp.dot(xnb, wqkv_ref[:, D:2 * D], preferred_element_type=_F32).astype(_BF16)
        kk = jnp.concatenate([kk, jnp.zeros((n, 128), _BF16)], axis=1)
        for w in range(_NG):
            k_scr[w, rows, :] = kk[:, w * GW:w * GW + 128]

    def proj_first(fn):
        for c0 in range(0, tp, tp0):
            fn(0, xn_scr[c0:c0 + tp0, :], c0)

    x_copy(0).wait()
    ln1(0)
    w_copy(0).wait()
    w_copy(2).start()
    w_copy(1).start()
    x_copy(1).start()
    proj_first(proj_q)
    w_copy(2).wait()
    for i in range(2, n_tp):
        x_copy(i).start()
    proj_first(proj_v)
    w_copy(1).wait()
    x_copy(1).wait()
    proj_first(proj_k)
    ln1(1)

    def proj(i, carry):
        @pl.when(i + 1 < n_tp)
        def _():
            x_copy(i + 1).wait()

        xnb = xn_scr[pl.ds(pl.multiple_of(i * tp, tp), tp), :]
        proj_q(i, xnb)
        proj_v(i, xnb)
        proj_k(i, xnb)
        ln1(jnp.minimum(i + 1, n_tp - 1))
        return carry

    lax.fori_loop(1, n_tp, proj, 0)
    for cp in late_copies:
        cp.start()

    def q_rhs(tt, g, j):
        r0 = pl.multiple_of(g * GW + 16 * j, 16)
        npc = tq // tp
        qt = [qT_scr[tt * npc + i, pl.ds(r0, 32), :] for i in range(npc)]
        qt = qt[0] if npc == 1 else jnp.concatenate(qt, axis=1)
        off = Dh * j - 16 * j
        r = lax.broadcasted_iota(jnp.int32, (32, tq), 0)
        qt = jnp.where(jnp.logical_and(r >= off, r < off + Dh), qt, jnp.zeros_like(qt))
        parts = []
        if j > 0:
            parts.append(jnp.zeros((16 * j, tq), _BF16))
        parts.append(qt)
        parts.append(jnp.zeros((128 - 32 - 16 * j, tq), _BF16))
        return jnp.concatenate(parts, axis=0)

    def a_chunk(g, rhs, c, buf, mrun):
        s = jnp.dot(k_scr[g, c * ck:(c + 1) * ck, :], rhs,
                    preferred_element_type=_F32)
        sb[buf][0, c * ck:(c + 1) * ck, :] = s
        mm = jnp.max(s.reshape(ck // 8, 8, tq), axis=0)
        return mm if mrun is None else jnp.maximum(mrun, mm)

    def v_block(j):
        b0 = ((Dh * j) // 8) * 8
        return b0, Dh * j - b0

    def b_chunk(g, j, c, buf, z, m, acc):
        p = jnp.exp2(sb[buf][z, c * ck:(c + 1) * ck, :] - m).astype(_BF16)
        b0, off = v_block(j)
        r0 = pl.multiple_of(g * GW + b0, 8)
        c0 = (c * ck) % tp
        vt = vT_scr[(c * ck) // tp, pl.ds(r0, 24), c0:c0 + ck]
        r = lax.broadcasted_iota(jnp.int32, (24, ck), 0)
        vl = jnp.where(jnp.logical_and(r >= off, r < off + Dh), vt, 1.0)
        o = lax.dot_general(vl, p, _NN, preferred_element_type=_F32)
        return o if acc is None else acc + o

    def b_finish(t, g, j, acc):
        b0, off = v_block(j)
        l = acc[0:1, :] if off > 0 else acc[23:24, :]
        on = acc * (1.0 / l)
        r0 = pl.multiple_of(g * GW + b0, 8)
        npr = tq // rs
        for i in range(npr):
            lo = on[0:8, i * rs:(i + 1) * rs]
            if off > 0:
                r = lax.broadcasted_iota(jnp.int32, (8, rs), 0)
                lo = jnp.where(r >= off, lo, oT_scr[t * npr + i, pl.ds(r0, 8), :])
            oT_scr[t * npr + i, pl.ds(r0, 8), :] = lo
            oT_scr[t * npr + i, pl.ds(r0 + 8, 16), :] = on[8:24, i * rs:(i + 1) * rs]

    z = zero_smem[0]
    gpi = unroll // _G

    def step(a_unit, b_unit, par):
        rhs = q_rhs(*a_unit)
        m = mb[1 - par][...]
        mrun = None
        acc = None
        for c in range(nck + skew):
            if c < nck:
                mrun = a_chunk(a_unit[1], rhs, c, par, mrun)
            if c >= skew:
                acc = b_chunk(b_unit[1], b_unit[2], c - skew, 1 - par, z, m, acc)
        mb[par][...] = jnp.max(mrun, axis=0, keepdims=True)
        b_finish(*b_unit, acc)

    def attn_body(it, carry):
        for gg in range(gpi):
            u = it * gpi + gg
            t = u // _NG
            g = u % _NG
            for j in range(_G):
                if j > 0:
                    b_unit = (t, g, j - 1)
                else:
                    up = jnp.maximum(u - 1, 0)
                    b_unit = (up // _NG, up % _NG, _G - 1)
                step((t, g, j), b_unit, j % 2)
        return carry

    lax.fori_loop(0, n_qt * _NG // gpi, attn_body, 0)

    for cp in late_copies:
        cp.wait()

    def out_proj(r, between=None):
        rows = pl.ds(pl.multiple_of(r * rs, rs), rs)
        o = oT_scr[r].astype(_BF16).T
        if between is None:
            att = jnp.dot(o, wo_ref[...], preferred_element_type=_F32)
        else:
            parts = []
            for n in range(D // 128):
                between(n)
                parts.append(jnp.dot(o, wo_ref[:, n * 128:(n + 1) * 128],
                                     preferred_element_type=_F32))
            between(D // 128)
            att = jnp.concatenate(parts, axis=1)
        h1 = x_ref[rows, :].astype(_F32) + att
        hn_scr[rows, :] = _layernorm_f32(h1).astype(_BF16)
        h1_scr[rows, :] = h1

    f_cuts = list(range(0, F, fc)) + [F]
    f_chunks = list(zip(f_cuts[:-1], f_cuts[1:]))
    f_chunks = f_chunks[-1:] + f_chunks[:-1]

    def act_chunk(hn, f0, f1):
        fa = f0 + ((f1 - f0) // 128) * 128
        g = lax.dot_general(hn, wgT_ref[f0:fa, :], _NT, preferred_element_type=_F32)
        u = lax.dot_general(hn, wuT_ref[f0:fa, :], _NT, preferred_element_type=_F32)
        a = (g * jax.nn.sigmoid(g) * u).astype(_BF16)
        if fa < f1:
            assert f1 - fa == 64
            w_t = jnp.concatenate([wgT_ref[fa:f1, :], wuT_ref[fa:f1, :]], axis=0)
            gu = lax.dot_general(hn, w_t, _NT, preferred_element_type=_F32)
            a_t = gu * jax.nn.sigmoid(gu) * pltpu.roll(gu, 64, axis=1)
            a = jnp.concatenate([a, a_t[:, 0:64].astype(_BF16)], axis=1)
        return a

    def ffn(row0, n, sem, mid_work=None):
        rows = pl.ds(pl.multiple_of(row0, n), n)
        hn = hn_scr[rows, :]
        y = h1_scr[rows, :]
        nfc = len(f_chunks)
        prev = None
        for c in range(nfc + 1):
            if c == mid and mid_work is not None:
                mid_work()
            a = act_chunk(hn, *f_chunks[c]) if c < nfc else None
            if prev is not None:
                f0, f1 = f_chunks[c - 1]
                y = y + jnp.dot(prev, wd_ref[f0:f1, :], preferred_element_type=_F32)
            prev = a
        out_scr[rows, :] = y.astype(out_scr.dtype)
        out_copy(row0, n, sem).start()

    ep = {"acc": None}
    m_last = m1[...]
    ep_cuts = [0, 2, 5, 8, 11, 14, nck]

    def ep_b(n):
        for c in range(ep_cuts[n], ep_cuts[n + 1]):
            ep["acc"] = b_chunk(_NG - 1, _G - 1, c, 1, z, m_last, ep["acc"])

    out_proj(0, ep_b)
    b_finish(n_qt - 1, _NG - 1, _G - 1, ep["acc"])

    n_main = n_rs - 1 if rt else n_rs

    def ffn_body(r, carry):
        ffn(r * rs, rs, r, lambda: out_proj(jnp.minimum(r + 1, n_rs - 1)))
        return carry

    lax.fori_loop(0, n_main, ffn_body, 0)
    if rt:
        def ffn_tail(i, carry):
            ffn(n_main * rs + i * rt, rt, n_main + i)
            return carry

        lax.fori_loop(0, rs // rt, ffn_tail, 0)
    for r in range(n_main):
        out_copy(r * rs, rs, r).wait()
    if rt:
        for i in range(rs // rt):
            out_copy(n_main * rs + i * rt, rt, n_main + i).wait()


def _build(S, D, F, dtype, tq=512, ck=128, unroll=8, tp=512, tp0=128, rs=256, rt=128, fc=256,
           mid=3, skew=2):
    assert tq % tp == 0 and tp % ck == 0 and tq % rs == 0 and S // ck == 16
    kern = functools.partial(_kernel, S=S, D=D, F=F, tq=tq, ck=ck, unroll=unroll, tp=tp, tp0=tp0,
                             rs=rs, rt=rt, fc=fc, mid=mid, skew=skew)
    n_out = S // rs + (rs // rt if rt else 0)
    return pl.pallas_call(
        kern,
        in_specs=[pl.BlockSpec(memory_space=pl.ANY)] * 6,
        out_specs=pl.BlockSpec(memory_space=pl.ANY),
        out_shape=jax.ShapeDtypeStruct((S, D), dtype),
        scratch_shapes=[
            pltpu.VMEM((S, D), _BF16),
            pltpu.VMEM((D, 3 * D), _BF16),
            pltpu.VMEM((D, D), _BF16),
            pltpu.VMEM((F, D), _BF16),
            pltpu.VMEM((F, D), _BF16),
            pltpu.VMEM((F, D), _BF16),
            pltpu.SemaphoreType.DMA((S // tp,)),
            pltpu.SemaphoreType.DMA((7,)),
            pltpu.SemaphoreType.DMA((n_out,)),
            pltpu.SMEM((1,), jnp.int32),
            pltpu.VMEM((S, D), _BF16),
            pltpu.VMEM((_NG, S, 128), _BF16),
            pltpu.VMEM((S // tp, D, tp), _BF16),
            pltpu.VMEM((S // tp, D, tp), _F32),
            pltpu.VMEM((1, S, tq), _F32),
            pltpu.VMEM((1, S, tq), _F32),
            pltpu.VMEM((1, tq), _F32),
            pltpu.VMEM((1, tq), _F32),
            pltpu.VMEM((S // rs, D, rs), _F32),
            pltpu.VMEM((S, D), _BF16),
            pltpu.VMEM((S, D), _F32),
            pltpu.VMEM((S, D), dtype),
        ],
        compiler_params=pltpu.CompilerParams(
            vmem_limit_bytes=100 * 1024 * 1024,
        ),
        name="preln_mha_swiglu",
    )


@jax.jit
def pallas_sequential_preLN__mha_block__swiglu_ffn__prompt_kernel(
    A_x: jax.Array,
    A_wqkv: jax.Array,
    A_wo: jax.Array,
    B_x: jax.Array,
    B_w_gate: jax.Array,
    B_w_up: jax.Array,
    B_w_down: jax.Array,
):
    B, S, D = A_x.shape
    F = B_w_gate.shape[1]
    assert B == 1 and D == 640 and S == 2048
    x = A_x.reshape(S, D)
    out = _build(S, D, F, A_x.dtype)(x, A_wqkv, A_wo, B_w_gate.T, B_w_up.T, B_w_down)
    return out.reshape(B, S, D)
```

```python
import functools
import math

import jax
import jax.numpy as jnp
from jax import lax
import jax.experimental.pallas as pl
import jax.experimental.pallas.tpu as pltpu

_H = 32
_EPS = 1e-5
_G = 4
_NG = _H // _G

_BF16 = jnp.bfloat16
_F32 = jnp.float32
_NT = (((1,), (1,)), ((), ()))
_NN = (((1,), (0,)), ((), ()))


def _layernorm_f32(x):
    m = jnp.mean(x, axis=-1, keepdims=True)
    xc = x - m
    v = jnp.mean(xc * xc, axis=-1, keepdims=True)
    return xc * lax.rsqrt(v + _EPS)


def _kernel(x_hbm, wqkv_hbm, wo_hbm, wgT_hbm, wuT_hbm, wd_hbm,
            out_hbm,
            x_ref, wqkv_ref, wo_ref, wgT_ref, wuT_ref, wd_ref,
            x_sems, w_sems, o_sems, zero_smem,
            xn_scr, k_scr, qT_scr, vT_scr, s0, s1, m0, m1, oT_scr,
            hn_scr, h1_scr, out_scr,
            *, S, D, F, tq, ck, unroll, tp, tp0, rs, rt, fc, mid, skew):
    Dh = D // _H
    n_qt = S // tq
    n_tp = S // tp
    n_rs = S // rs
    nck = S // ck
    GW = _G * Dh
    sb = (s0, s1)
    mb = (m0, m1)

    def x_copy(i):
        rows = pl.ds(pl.multiple_of(i * tp, tp), tp)
        return pltpu.make_async_copy(x_hbm.at[rows, :], x_ref.at[rows, :], x_sems.at[i])

    def w_copy(i):
        cols = pl.ds(i * D, D)
        return pltpu.make_async_copy(wqkv_hbm.at[:, cols], wqkv_ref.at[:, cols], w_sems.at[i])

    late_copies = [
        pltpu.make_async_copy(wo_hbm, wo_ref, w_sems.at[3]),
        pltpu.make_async_copy(wgT_hbm, wgT_ref, w_sems.at[4]),
        pltpu.make_async_copy(wuT_hbm, wuT_ref, w_sems.at[5]),
        pltpu.make_async_copy(wd_hbm, wd_ref, w_sems.at[6]),
    ]

    def out_copy(row0, n, sem):
        rows = pl.ds(pl.multiple_of(row0, n), n)
        return pltpu.make_async_copy(out_scr.at[rows, :], out_hbm.at[rows, :], o_sems.at[sem])

    x_copy(0).start()
    w_copy(0).start()
    zero_smem[0] = 0

    def zero_fill(i, carry):
        s1[0, pl.ds(pl.multiple_of(i * ck, ck), ck), :] = jnp.zeros((ck, tq), _F32)
        return carry

    lax.fori_loop(0, nck, zero_fill, 0)
    m1[...] = jnp.zeros_like(m1)
    oT_scr[0:tq // rs, 0:GW, :] = jnp.zeros((tq // rs, GW, rs), _F32)

    def ln1(i, c0=0, n=tp):
        rows = pl.ds(pl.multiple_of(i * tp + c0, n), n)
        xn_scr[rows, :] = _layernorm_f32(x_ref[rows, :].astype(_F32)).astype(_BF16)

    qscale = (Dh ** -0.5) * math.log2(math.e)

    def proj_q(i, xnb, c0=0):
        n = xnb.shape[0]
        q = jnp.dot(xnb, wqkv_ref[:, 0:D], preferred_element_type=_F32) * qscale
        qT_scr[i, :, c0:c0 + n] = q.astype(_BF16).T

    def proj_v(i, xnb, c0=0):
        n = xnb.shape[0]
        v = jnp.dot(xnb, wqkv_ref[:, 2 * D:3 * D], preferred_element_type=_F32)
        vT_scr[i, :, c0:c0 + n] = v.astype(_BF16).T.astype(_F32)

    def proj_k(i, xnb, c0=0):
        n = xnb.shape[0]
        rows = pl.ds(pl.multiple_of(i * tp + c0, 128), n)
        kk = jnp.dot(xnb, wqkv_ref[:, D:2 * D], preferred_element_type=_F32).astype(_BF16)
        kk = jnp.concatenate([kk, jnp.zeros((n, 128), _BF16)], axis=1)
        for w in range(_NG):
            k_scr[w, rows, :] = kk[:, w * GW:w * GW + 128]

    def proj_first(fn):
        for c0 in range(0, tp, tp0):
            fn(0, xn_scr[c0:c0 + tp0, :], c0)

    x_copy(0).wait()
    ln1(0)
    w_copy(0).wait()
    w_copy(2).start()
    w_copy(1).start()
    x_copy(1).start()
    proj_first(proj_q)
    w_copy(2).wait()
    for i in range(2, n_tp):
        x_copy(i).start()
    proj_first(proj_v)
    w_copy(1).wait()
    x_copy(1).wait()
    for c0 in range(0, tp, tp0):
        proj_k(0, xn_scr[c0:c0 + tp0, :], c0)
        ln1(1, c0, tp0)

    def proj(i, carry):
        @pl.when(i + 1 < n_tp)
        def _():
            x_copy(i + 1).wait()

        xnb = xn_scr[pl.ds(pl.multiple_of(i * tp, tp), tp), :]
        proj_q(i, xnb)
        proj_v(i, xnb)
        proj_k(i, xnb)
        ln1(jnp.minimum(i + 1, n_tp - 1))
        return carry

    lax.fori_loop(1, n_tp, proj, 0)
    for cp in late_copies:
        cp.start()

    def q_rhs(tt, g, j):
        r0 = pl.multiple_of(g * GW + 16 * j, 16)
        npc = tq // tp
        qt = [qT_scr[tt * npc + i, pl.ds(r0, 32), :] for i in range(npc)]
        qt = qt[0] if npc == 1 else jnp.concatenate(qt, axis=1)
        off = Dh * j - 16 * j
        r = lax.broadcasted_iota(jnp.int32, (32, tq), 0)
        qt = jnp.where(jnp.logical_and(r >= off, r < off + Dh), qt, jnp.zeros_like(qt))
        parts = []
        if j > 0:
            parts.append(jnp.zeros((16 * j, tq), _BF16))
        parts.append(qt)
        parts.append(jnp.zeros((128 - 32 - 16 * j, tq), _BF16))
        return jnp.concatenate(parts, axis=0)

    def a_chunk(g, rhs, c, buf, mrun):
        s = jnp.dot(k_scr[g, c * ck:(c + 1) * ck, :], rhs,
                    preferred_element_type=_F32)
        sb[buf][0, c * ck:(c + 1) * ck, :] = s
        mm = jnp.max(s.reshape(ck // 8, 8, tq), axis=0)
        return mm if mrun is None else jnp.maximum(mrun, mm)

    def v_block(j):
        b0 = ((Dh * j) // 8) * 8
        return b0, Dh * j - b0

    def b_chunk(g, j, c, buf, z, m, acc):
        p = jnp.exp2(sb[buf][z, c * ck:(c + 1) * ck, :] - m).astype(_BF16)
        b0, off = v_block(j)
        r0 = pl.multiple_of(g * GW + b0, 8)
        c0 = (c * ck) % tp
        vt = vT_scr[(c * ck) // tp, pl.ds(r0, 24), c0:c0 + ck]
        r = lax.broadcasted_iota(jnp.int32, (24, ck), 0)
        vl = jnp.where(jnp.logical_and(r >= off, r < off + Dh), vt, 1.0)
        o = lax.dot_general(vl, p, _NN, preferred_element_type=_F32)
        return o if acc is None else acc + o

    def b_finish(t, g, j, acc):
        b0, off = v_block(j)
        l = acc[0:1, :] if off > 0 else acc[23:24, :]
        on = acc * (1.0 / l)
        r0 = pl.multiple_of(g * GW + b0, 8)
        npr = tq // rs
        for i in range(npr):
            lo = on[0:8, i * rs:(i + 1) * rs]
            if off > 0:
                r = lax.broadcasted_iota(jnp.int32, (8, rs), 0)
                lo = jnp.where(r >= off, lo, oT_scr[t * npr + i, pl.ds(r0, 8), :])
            oT_scr[t * npr + i, pl.ds(r0, 8), :] = lo
            oT_scr[t * npr + i, pl.ds(r0 + 8, 16), :] = on[8:24, i * rs:(i + 1) * rs]

    z = zero_smem[0]
    gpi = unroll // _G

    def step(a_unit, b_unit, par):
        rhs = q_rhs(*a_unit)
        m = mb[1 - par][...]
        mrun = None
        acc = None
        for c in range(nck + skew):
            if c < nck:
                mrun = a_chunk(a_unit[1], rhs, c, par, mrun)
            if c >= skew:
                acc = b_chunk(b_unit[1], b_unit[2], c - skew, 1 - par, z, m, acc)
        mb[par][...] = jnp.max(mrun, axis=0, keepdims=True)
        b_finish(*b_unit, acc)

    def attn_body(it, carry):
        for gg in range(gpi):
            u = it * gpi + gg
            t = u // _NG
            g = u % _NG
            for j in range(_G):
                if j > 0:
                    b_unit = (t, g, j - 1)
                else:
                    up = jnp.maximum(u - 1, 0)
                    b_unit = (up // _NG, up % _NG, _G - 1)
                step((t, g, j), b_unit, j % 2)
        return carry

    lax.fori_loop(0, n_qt * _NG // gpi, attn_body, 0)

    for cp in late_copies:
        cp.wait()

    def out_proj(r, between=None):
        rows = pl.ds(pl.multiple_of(r * rs, rs), rs)
        o = oT_scr[r].astype(_BF16).T
        if between is None:
            att = jnp.dot(o, wo_ref[...], preferred_element_type=_F32)
        else:
            parts = []
            for n in range(D // 128):
                between(n)
                parts.append(jnp.dot(o, wo_ref[:, n * 128:(n + 1) * 128],
                                     preferred_element_type=_F32))
            between(D // 128)
            att = jnp.concatenate(parts, axis=1)
        h1 = x_ref[rows, :].astype(_F32) + att
        hn_scr[rows, :] = _layernorm_f32(h1).astype(_BF16)
        h1_scr[rows, :] = h1

    f_cuts = list(range(0, F, fc)) + [F]
    f_chunks = list(zip(f_cuts[:-1], f_cuts[1:]))
    f_chunks = f_chunks[-1:] + f_chunks[:-1]

    def act_chunk(hn, f0, f1):
        fa = f0 + ((f1 - f0) // 128) * 128
        g = lax.dot_general(hn, wgT_ref[f0:fa, :], _NT, preferred_element_type=_F32)
        u = lax.dot_general(hn, wuT_ref[f0:fa, :], _NT, preferred_element_type=_F32)
        a = (g * jax.nn.sigmoid(g) * u).astype(_BF16)
        if fa < f1:
            assert f1 - fa == 64
            w_t = jnp.concatenate([wgT_ref[fa:f1, :], wuT_ref[fa:f1, :]], axis=0)
            gu = lax.dot_general(hn, w_t, _NT, preferred_element_type=_F32)
            a_t = gu * jax.nn.sigmoid(gu) * pltpu.roll(gu, 64, axis=1)
            a = jnp.concatenate([a, a_t[:, 0:64].astype(_BF16)], axis=1)
        return a

    def ffn(row0, n, sem, mid_work=None):
        rows = pl.ds(pl.multiple_of(row0, n), n)
        hn = hn_scr[rows, :]
        y = h1_scr[rows, :]
        nfc = len(f_chunks)
        prev = None
        for c in range(nfc + 1):
            if c == mid and mid_work is not None:
                mid_work()
            a = act_chunk(hn, *f_chunks[c]) if c < nfc else None
            if prev is not None:
                f0, f1 = f_chunks[c - 1]
                y = y + jnp.dot(prev, wd_ref[f0:f1, :], preferred_element_type=_F32)
            prev = a
        out_scr[rows, :] = y.astype(out_scr.dtype)
        out_copy(row0, n, sem).start()

    ep = {"acc": None}
    m_last = m1[...]
    ep_cuts = [0, 2, 5, 8, 11, 14, nck]

    def ep_b(n):
        for c in range(ep_cuts[n], ep_cuts[n + 1]):
            ep["acc"] = b_chunk(_NG - 1, _G - 1, c, 1, z, m_last, ep["acc"])

    out_proj(0, ep_b)
    b_finish(n_qt - 1, _NG - 1, _G - 1, ep["acc"])

    n_main = n_rs - 1 if rt else n_rs

    def ffn_body(r, carry):
        ffn(r * rs, rs, r, lambda: out_proj(jnp.minimum(r + 1, n_rs - 1)))
        return carry

    lax.fori_loop(0, n_main, ffn_body, 0)
    if rt:
        def ffn_tail(i, carry):
            ffn(n_main * rs + i * rt, rt, n_main + i)
            return carry

        lax.fori_loop(0, rs // rt, ffn_tail, 0)
    for r in range(n_main):
        out_copy(r * rs, rs, r).wait()
    if rt:
        for i in range(rs // rt):
            out_copy(n_main * rs + i * rt, rt, n_main + i).wait()


def _build(S, D, F, dtype, tq=512, ck=128, unroll=8, tp=512, tp0=128, rs=256, rt=128, fc=256,
           mid=4, skew=2):
    assert tq % tp == 0 and tp % ck == 0 and tq % rs == 0 and S // ck == 16
    kern = functools.partial(_kernel, S=S, D=D, F=F, tq=tq, ck=ck, unroll=unroll, tp=tp, tp0=tp0,
                             rs=rs, rt=rt, fc=fc, mid=mid, skew=skew)
    n_out = S // rs + (rs // rt if rt else 0)
    return pl.pallas_call(
        kern,
        in_specs=[pl.BlockSpec(memory_space=pl.ANY)] * 6,
        out_specs=pl.BlockSpec(memory_space=pl.ANY),
        out_shape=jax.ShapeDtypeStruct((S, D), dtype),
        scratch_shapes=[
            pltpu.VMEM((S, D), _BF16),
            pltpu.VMEM((D, 3 * D), _BF16),
            pltpu.VMEM((D, D), _BF16),
            pltpu.VMEM((F, D), _BF16),
            pltpu.VMEM((F, D), _BF16),
            pltpu.VMEM((F, D), _BF16),
            pltpu.SemaphoreType.DMA((S // tp,)),
            pltpu.SemaphoreType.DMA((7,)),
            pltpu.SemaphoreType.DMA((n_out,)),
            pltpu.SMEM((1,), jnp.int32),
            pltpu.VMEM((S, D), _BF16),
            pltpu.VMEM((_NG, S, 128), _BF16),
            pltpu.VMEM((S // tp, D, tp), _BF16),
            pltpu.VMEM((S // tp, D, tp), _F32),
            pltpu.VMEM((1, S, tq), _F32),
            pltpu.VMEM((1, S, tq), _F32),
            pltpu.VMEM((1, tq), _F32),
            pltpu.VMEM((1, tq), _F32),
            pltpu.VMEM((S // rs, D, rs), _F32),
            pltpu.VMEM((S, D), _BF16),
            pltpu.VMEM((S, D), _F32),
            pltpu.VMEM((S, D), dtype),
        ],
        compiler_params=pltpu.CompilerParams(
            vmem_limit_bytes=100 * 1024 * 1024,
        ),
        name="preln_mha_swiglu",
    )


@jax.jit
def pallas_sequential_preLN__mha_block__swiglu_ffn__prompt_kernel(
    A_x: jax.Array,
    A_wqkv: jax.Array,
    A_wo: jax.Array,
    B_x: jax.Array,
    B_w_gate: jax.Array,
    B_w_up: jax.Array,
    B_w_down: jax.Array,
):
    B, S, D = A_x.shape
    F = B_w_gate.shape[1]
    assert B == 1 and D == 640 and S == 2048
    x = A_x.reshape(S, D)
    out = _build(S, D, F, A_x.dtype)(x, A_wqkv, A_wo, B_w_gate.T, B_w_up.T, B_w_down)
    return out.reshape(B, S, D)
```
